```python
import jax
import jax.numpy as jnp

def _softmax(x, axis=-1):
    return jax.nn.softmax(x, axis=axis)
def _gelu(x):
    return jax.nn.gelu(x, approximate=True)
def _silu(x):
    return jax.nn.silu(x)
def _sigmoid(x):
    return jax.nn.sigmoid(x)
def _layernorm(x, axis=-1, eps=1e-5):
    m = jnp.mean(x, axis=axis, keepdims=True)
    v = jnp.var(x, axis=axis, keepdims=True)
    return (x - m) / jnp.sqrt(v + eps)
def _scatter_add(tgt, idx, src, axis=0):
    return tgt.at[idx].add(src)
def _segment_sum(src, seg, n):
    return jax.ops.segment_sum(src, seg, n)
class _Rng:
    def __init__(self, key):
        self._k = key
    def _next(self):
        self._k, sub = jax.random.split(self._k)
        return sub
    def normal(self, shape):
        return jax.random.normal(self._next(), shape, dtype=jnp.bfloat16)
    def randint(self, lo, hi, shape):
        return jax.random.randint(self._next(), shape, lo, hi, dtype=jnp.int32)
    def uniform(self, shape, lo=0.0, hi=1.0):
        return jax.random.uniform(self._next(), shape, jnp.bfloat16, lo, hi)
    def permutation(self, n):
        return jax.random.permutation(self._next(), n)


kernel_name = 'interleave_layers__sliding_local_dilated__glu_gated_bilinear__prompt'

def setup_inputs():
    _rng = _Rng(jax.random.key(int.from_bytes(__import__("os").urandom(4), "little")))
    _w = (lambda a: (lambda t: t.astype(jnp.bfloat16) if jnp.issubdtype(t.dtype, jnp.floating) else t)(jnp.asarray(a)))
    def _A_setup():
        B, S, D = 1, 2048, 576
        return {
            "x": _w((lambda *s: _rng.normal(s) * 0.05)(B, S, D)),
            "wqkv": _w((lambda *s: _rng.normal(s) * 0.05)(D, 3 * D)),
            "wo": _w((lambda *s: _rng.normal(s) * 0.05)(D, D)),
        }
    _A_in = _A_setup()

    def _B_setup():
        B, S, D, F = 1, 2048, 576, 4608
        return {
            "x": _w((lambda *s: _rng.normal(s) * 0.05)(B, S, D)),
            "w_gate": _w((lambda *s: _rng.normal(s) * 0.05)(D, F) * (D ** -0.5)),
            "w_up": _w((lambda *s: _rng.normal(s) * 0.05)(D, F) * (D ** -0.5)),
            "w_down": _w((lambda *s: _rng.normal(s) * 0.05)(F, D) * (F ** -0.5)),
        }
    _B_in = _B_setup()

    return {
        "A_x": _A_in["x"],
        "A_wqkv": _A_in["wqkv"],
        "A_wo": _A_in["wo"],
        "B_x": _B_in["x"],
        "B_w_gate": _B_in["w_gate"],
        "B_w_up": _B_in["w_up"],
        "B_w_down": _B_in["w_down"],
    }

def reference(A_x, A_wqkv, A_wo, B_x, B_w_gate, B_w_up, B_w_down):
    def _A_ref(x, wqkv, wo):
        B, S, D = x.shape
        H = 32; Dh = D // H
        W, dil = 8, 2
        qkv = (lambda x, *d: x.transpose(*d))((x @ wqkv).reshape(B, S, 3, H, Dh), 2, 0, 3, 1, 4)
        q, k, v = qkv[0], qkv[1], qkv[2]
        scale = Dh ** -0.5
        pos = jnp.arange(S)
        off = jnp.arange(W) * dil
        idx = pos[:, None] - off[None, :]
        mask = idx >= 0
        idx_c = jnp.where(mask, idx, 0).reshape(-1)
        kg = k[:, :, idx_c, :].reshape(B, H, S, W, Dh)
        vg = v[:, :, idx_c, :].reshape(B, H, S, W, Dh)
        logits = jnp.einsum("bhsd,bhswd->bhsw", q, kg) * scale
        logits = jnp.where(mask[None, None, :, :], logits, -1e9)
        attn = _softmax(logits, axis=-1)
        o = jnp.einsum("bhsw,bhswd->bhsd", attn, vg)
        return (lambda x, *d: x.transpose(*d))(o, 0, 2, 1, 3).reshape(B, S, D) @ wo

    def _B_ref(x, w_gate, w_up, w_down):
        g = jnp.einsum("bsd,df->bsf", x, w_gate)
        u = jnp.einsum("bsd,df->bsf", x, w_up)
        h = g * u
        return jnp.einsum("bsf,fd->bsd", h, w_down)

    x = A_x
    x = x + _A_ref(_layernorm(x, axis=-1), A_wqkv, A_wo)
    x = x + _B_ref(_layernorm(x, axis=-1), B_w_gate, B_w_up, B_w_down)
    x = x + _A_ref(_layernorm(x, axis=-1), A_wqkv, A_wo)
    x = x + _B_ref(_layernorm(x, axis=-1), B_w_gate, B_w_up, B_w_down)
    return x
```

```python
import jax
import jax.numpy as jnp
import jax.experimental.pallas as pl
import jax.experimental.pallas.tpu as pltpu

S = 2048
D = 576
DP = 640
F = 4608
H = 32
DH = 18
W = 8
DIL = 2
HALO = 16
TA = 256
TB = 512
FC = 768
EPS = 1e-5


def _ln_t(xt):
    m = jnp.mean(xt, axis=0, keepdims=True)
    xc = xt - m
    v = jnp.mean(xc * xc, axis=0, keepdims=True)
    return (xc * jax.lax.rsqrt(v + EPS)).T.astype(jnp.bfloat16)


_NT = (((1,), (1,)), ((), ()))


def _kernel(x_hbm, wqkv_hbm, wo_hbm, wg_hbm, wu_hbm, wd_hbm, out_hbm,
            xin, wqkv_raw, wo_raw, wqkv_p, wo_p, wg, wu, wd,
            xres, qbuf, kbuf, vbuf, outb, sems):
    cp_wqkv = pltpu.make_async_copy(wqkv_hbm, wqkv_raw, sems.at[0])
    cp_x = pltpu.make_async_copy(x_hbm, xin, sems.at[1])
    cp_wo = pltpu.make_async_copy(wo_hbm, wo_raw, sems.at[2])
    cp_wg = pltpu.make_async_copy(wg_hbm, wg, sems.at[3])
    cp_wu = pltpu.make_async_copy(wu_hbm, wu, sems.at[4])
    cp_wd = pltpu.make_async_copy(wd_hbm, wd, sems.at[5])
    cp_wqkv.start()
    cp_x.start()
    cp_wo.start()
    cp_wg.start()
    cp_wu.start()
    cp_wd.start()

    r = jax.lax.broadcasted_iota(jnp.int32, (D, DP), 0)
    j = jax.lax.broadcasted_iota(jnp.int32, (D, DP), 1)
    perm = jnp.where((r == (j % H) * DH + j // H) & (j < D), 1.0, 0.0).astype(jnp.bfloat16)

    kbuf[0:HALO, :] = jnp.zeros((HALO, DP), jnp.float32)
    vbuf[0:HALO, :] = jnp.zeros((HALO, DP), jnp.float32)

    cp_wqkv.wait()
    for c in range(3):
        wc = wqkv_raw[:, c * D:(c + 1) * D]
        wqkv_p[:, c * DP:(c + 1) * DP] = jnp.dot(
            wc, perm, preferred_element_type=jnp.float32).astype(jnp.bfloat16)
    cp_wo.wait()
    wo_p[...] = jax.lax.dot_general(
        wo_raw[...], perm, (((0,), (0,)), ((), ())),
        preferred_element_type=jnp.float32).astype(jnp.bfloat16)
    cp_x.wait()

    scale = DH ** -0.5

    def attn_tile(i, src_ref):
        r0 = pl.multiple_of(i * TA, TA)
        x = src_ref[:, pl.ds(r0, TA)].astype(jnp.float32)
        xn = _ln_t(x)
        qkv = jnp.dot(xn, wqkv_p[...], preferred_element_type=jnp.float32)
        qbuf[...] = qkv[:, 0:DP] * scale
        kbuf[HALO:HALO + TA, :] = qkv[:, DP:2 * DP]
        vbuf[HALO:HALO + TA, :] = qkv[:, 2 * DP:3 * DP]
        rows = r0 + jax.lax.broadcasted_iota(jnp.int32, (TA, 128), 0)
        logits = []
        for w in range(W):
            o = HALO - DIL * w
            acc = None
            for t in range(DP // 128):
                pr = qbuf[:, t * 128:(t + 1) * 128] * kbuf[o:o + TA, t * 128:(t + 1) * 128]
                acc = pr if acc is None else acc + pr
            acc = acc + pltpu.roll(acc, 64, 1)
            acc = acc + pltpu.roll(acc, 32, 1)
            if w > 0:
                acc = jnp.where(rows >= DIL * w, acc, -1e9)
            logits.append(acc)
        m = logits[0]
        for w in range(1, W):
            m = jnp.maximum(m, logits[w])
        ps = [jnp.exp(l - m) for l in logits]
        den = ps[0]
        for w in range(1, W):
            den = den + ps[w]
        inv = 1.0 / den
        os_ = []
        for t in range(DP // 128):
            acc = None
            for w in range(W):
                o = HALO - DIL * w
                pr = ps[w] * vbuf[o:o + TA, t * 128:(t + 1) * 128]
                acc = pr if acc is None else acc + pr
            os_.append((acc * inv).astype(jnp.bfloat16))
        ob = jnp.concatenate(os_, axis=1)
        y = jax.lax.dot_general(wo_p[...], ob, _NT, preferred_element_type=jnp.float32)
        xres[:, pl.ds(r0, TA)] = x + y
        kbuf[0:HALO, :] = kbuf[TA:TA + HALO, :]
        vbuf[0:HALO, :] = vbuf[TA:TA + HALO, :]

    def ffn_tile(i, last):
        r0 = pl.multiple_of(i * TB, TB)
        x = xres[:, pl.ds(r0, TB)]
        xn = _ln_t(x)
        acc = x
        for c in range(F // FC):
            sl = slice(c * FC, (c + 1) * FC)
            g = jnp.dot(xn, wg[:, sl], preferred_element_type=jnp.float32)
            u = jnp.dot(xn, wu[:, sl], preferred_element_type=jnp.float32)
            h = (g * u).astype(jnp.bfloat16)
            acc = acc + jax.lax.dot_general(wd[:, sl], h, _NT,
                                            preferred_element_type=jnp.float32)
        if last:
            outb[:, pl.ds(r0, TB)] = acc.astype(jnp.bfloat16)
        else:
            xres[:, pl.ds(r0, TB)] = acc

    for layer in range(2):
        src = xin if layer == 0 else xres

        @pl.loop(0, S // TA)
        def _(i):
            attn_tile(i, src)

        if layer == 0:
            cp_wg.wait()
            cp_wu.wait()
            cp_wd.wait()
            kbuf[0:HALO, :] = jnp.zeros((HALO, DP), jnp.float32)
            vbuf[0:HALO, :] = jnp.zeros((HALO, DP), jnp.float32)

        @pl.loop(0, S // TB)
        def _(i):
            ffn_tile(i, layer == 1)

    cp_out = pltpu.make_async_copy(outb, out_hbm, sems.at[6])
    cp_out.start()
    cp_out.wait()


@jax.jit
def pallas_interleave_layers__sliding_local_dilated__glu_gated_bilinear__prompt_kernel(
    A_x: jax.Array,
    A_wqkv: jax.Array,
    A_wo: jax.Array,
    B_x: jax.Array,
    B_w_gate: jax.Array,
    B_w_up: jax.Array,
    B_w_down: jax.Array,
):
    x2 = A_x.reshape(S, D).T
    bf = jnp.bfloat16
    f32 = jnp.float32
    out = pl.pallas_call(
        _kernel,
        out_shape=jax.ShapeDtypeStruct((D, S), bf),
        in_specs=[pl.BlockSpec(memory_space=pltpu.HBM)] * 6,
        out_specs=pl.BlockSpec(memory_space=pltpu.HBM),
        scratch_shapes=[
            pltpu.VMEM((D, S), bf),
            pltpu.VMEM((D, 3 * D), bf),
            pltpu.VMEM((D, D), bf),
            pltpu.VMEM((D, 3 * DP), bf),
            pltpu.VMEM((D, DP), bf),
            pltpu.VMEM((D, F), bf),
            pltpu.VMEM((D, F), bf),
            pltpu.VMEM((D, F), bf),
            pltpu.VMEM((D, S), f32),
            pltpu.VMEM((TA, DP), f32),
            pltpu.VMEM((TA + HALO, DP), f32),
            pltpu.VMEM((TA + HALO, DP), f32),
            pltpu.VMEM((D, S), bf),
            pltpu.SemaphoreType.DMA((8,)),
        ],
        compiler_params=pltpu.CompilerParams(vmem_limit_bytes=100 * 1024 * 1024),
    )(x2, A_wqkv, A_wo, B_w_gate, B_w_up, B_w_down.T)
    return out.T.reshape(1, S, D)
```

```python
import jax
import jax.numpy as jnp
import jax.experimental.pallas as pl
import jax.experimental.pallas.tpu as pltpu

S = 2048
D = 576
DP = 640
F = 4608
H = 32
DH = 18
W = 8
DIL = 2
HALO = 16
T = 256
NT = S // T
LEAD = 2
FC = 768
SCHED = "ab" + "bababababab"
EPS = 1e-5


def _ln_t(xt):
    m = jnp.mean(xt, axis=0, keepdims=True)
    xc = xt - m
    v = jnp.mean(xc * xc, axis=0, keepdims=True)
    return (xc * jax.lax.rsqrt(v + EPS)).T.astype(jnp.bfloat16)


_NT = (((1,), (1,)), ((), ()))


def _kernel(x_hbm, wqkv_hbm, wo_hbm, wg_hbm, wu_hbm, wd_hbm, out_hbm,
            xin, wqkv_raw, wo_raw, wqkv_p, wo_p, wg, wu, wd,
            xres, xnb, qbuf, kbuf, vbuf, outb, sems):
    cp_wqkv = pltpu.make_async_copy(wqkv_hbm, wqkv_raw, sems.at[0])
    cp_x = pltpu.make_async_copy(x_hbm, xin, sems.at[1])
    cp_wo = pltpu.make_async_copy(wo_hbm, wo_raw, sems.at[2])
    cp_wg = pltpu.make_async_copy(wg_hbm, wg, sems.at[3])
    cp_wu = pltpu.make_async_copy(wu_hbm, wu, sems.at[4])
    cp_wd = pltpu.make_async_copy(wd_hbm, wd, sems.at[5])
    cp_wqkv.start()
    cp_x.start()
    cp_wo.start()
    cp_wg.start()
    cp_wu.start()
    cp_wd.start()

    r = jax.lax.broadcasted_iota(jnp.int32, (D, DP), 0)
    j = jax.lax.broadcasted_iota(jnp.int32, (D, DP), 1)
    perm = jnp.where((r == (j % H) * DH + j // H) & (j < D), 1.0, 0.0).astype(jnp.bfloat16)

    cp_wqkv.wait()
    r2 = jax.lax.broadcasted_iota(jnp.int32, (D, 128), 0)
    j2 = jax.lax.broadcasted_iota(jnp.int32, (D, 128), 1) + (512 - 64)
    perm_hi = jnp.where((r2 == (j2 % H) * DH + j2 // H) & (j2 >= 512),
                        1.0, 0.0).astype(jnp.bfloat16)
    rest = []
    for c in range(3):
        wc = wqkv_raw[:, c * D:(c + 1) * D]
        wqkv_p[:, c * 512:(c + 1) * 512] = jnp.dot(
            wc, perm[:, :512], preferred_element_type=jnp.float32).astype(jnp.bfloat16)
        rest.append(jnp.dot(wc, perm_hi if c == 2 else perm[:, 512:],
                            preferred_element_type=jnp.float32))
    wqkv_p[:, 1536:1664] = (rest[0] + rest[2]).astype(jnp.bfloat16)
    wqkv_p[:, 1664:1792] = rest[1].astype(jnp.bfloat16)
    cp_wo.wait()
    wo_p[...] = jax.lax.dot_general(
        wo_raw[...], jnp.concatenate([perm[:, :512], perm_hi], axis=1),
        (((0,), (0,)), ((), ())),
        preferred_element_type=jnp.float32).astype(jnp.bfloat16)
    cp_x.wait()

    scale = DH ** -0.5

    @pl.loop(0, NT)
    def _(i):
        c0 = pl.multiple_of(i * T, T)
        xres[:, pl.ds(c0, T)] = xin[:, pl.ds(c0, T)].astype(jnp.float32)

    def attn_tile(n):
        i = n % NT
        c0 = pl.multiple_of(i * T, T)
        x = xres[:, pl.ds(c0, T)]
        yield
        xn = _ln_t(x)
        qkv = jnp.dot(xn, wqkv_p[...], preferred_element_type=jnp.float32)
        qbuf[:, 0:512] = qkv[:, 0:512] * scale
        qbuf[:, 512:DP] = qkv[:, 1536:1664] * scale
        kbuf[0:HALO, :] = jnp.where(i > 0, kbuf[T:T + HALO, :], 0.0)
        vbuf[0:HALO, :] = jnp.where(i > 0, vbuf[T:T + HALO, :], 0.0)
        kbuf[HALO:HALO + T, 0:512] = qkv[:, 512:1024]
        kbuf[HALO:HALO + T, 512:DP] = qkv[:, 1664:1792]
        vbuf[HALO:HALO + T, 0:512] = qkv[:, 1024:1536]
        vbuf[HALO:HALO + T, 512:DP] = qkv[:, 1536:1664]
        rows = c0 + jax.lax.broadcasted_iota(jnp.int32, (T, 128), 0)
        logits = []
        for w in range(W):
            o = HALO - DIL * w
            acc = None
            for t in range(DP // 128):
                pr = qbuf[:, t * 128:(t + 1) * 128] * kbuf[o:o + T, t * 128:(t + 1) * 128]
                acc = pr if acc is None else acc + pr
            acc = acc + pltpu.roll(acc, 64, 1)
            acc = acc + pltpu.roll(acc, 32, 1)
            if w > 0:
                acc = jnp.where(rows >= DIL * w, acc, -1e9)
            logits.append(acc)
            if w % 4 == 3:
                yield
        m = logits[0]
        for w in range(1, W):
            m = jnp.maximum(m, logits[w])
        ps = [jnp.exp(l - m) for l in logits]
        den = ps[0]
        for w in range(1, W):
            den = den + ps[w]
        inv = 1.0 / den
        os_ = []
        for t in range(DP // 128):
            acc = None
            for w in range(W):
                o = HALO - DIL * w
                pr = ps[w] * vbuf[o:o + T, t * 128:(t + 1) * 128]
                acc = pr if acc is None else acc + pr
            os_.append((acc * inv).astype(jnp.bfloat16))
            if t == 2:
                yield
        yield
        ob = jnp.concatenate(os_, axis=1)
        y = jax.lax.dot_general(wo_p[...], ob, _NT, preferred_element_type=jnp.float32)
        x2 = x + y
        xn2 = _ln_t(x2)
        yield
        xres[:, pl.ds(c0, T)] = x2
        xnb[pl.ds(c0, T), :] = xn2

    def ffn_tile(n):
        i = n % NT
        c0 = pl.multiple_of(i * T, T)
        xn = xnb[pl.ds(c0, T), :]
        acc = xres[:, pl.ds(c0, T)]
        yield
        for c in range(F // FC):
            sl = slice(c * FC, (c + 1) * FC)
            g = jnp.dot(xn, wg[:, sl], preferred_element_type=jnp.float32)
            u = jnp.dot(xn, wu[:, sl], preferred_element_type=jnp.float32)
            h = (g * u).astype(jnp.bfloat16)
            acc = acc + jax.lax.dot_general(wd[:, sl], h, _NT,
                                            preferred_element_type=jnp.float32)
            yield
        xres[:, pl.ds(c0, T)] = acc
        outb[:, pl.ds(c0, T)] = acc.astype(jnp.bfloat16)

    def out_copy(i):
        c0 = pl.multiple_of(i * T, T)
        return pltpu.make_async_copy(outb.at[:, pl.ds(c0, T)],
                                     out_hbm.at[:, pl.ds(c0, T)], sems.at[6])

    kbuf[T:T + HALO, :] = jnp.zeros((HALO, DP), jnp.float32)
    vbuf[T:T + HALO, :] = jnp.zeros((HALO, DP), jnp.float32)

    @pl.loop(0, LEAD)
    def _(n):
        for _ in attn_tile(n):
            pass

    cp_wg.wait()
    cp_wu.wait()
    cp_wd.wait()

    @pl.loop(LEAD, 2 * NT)
    def _(n):
        a = attn_tile(n)
        b = ffn_tile(n - LEAD)
        for ch in SCHED:
            next(a if ch == "a" else b, None)
        for _ in a:
            pass
        for _ in b:
            pass

        @pl.when(n - LEAD >= NT)
        def _():
            out_copy(n - LEAD - NT).start()

    @pl.loop(2 * NT - LEAD, 2 * NT)
    def _(n):
        for _ in ffn_tile(n):
            pass
        out_copy(n - NT).start()

    @pl.loop(0, NT)
    def _(i):
        out_copy(i).wait()


@jax.jit
def pallas_interleave_layers__sliding_local_dilated__glu_gated_bilinear__prompt_kernel(
    A_x: jax.Array,
    A_wqkv: jax.Array,
    A_wo: jax.Array,
    B_x: jax.Array,
    B_w_gate: jax.Array,
    B_w_up: jax.Array,
    B_w_down: jax.Array,
):
    x2 = A_x.reshape(S, D).T
    bf = jnp.bfloat16
    f32 = jnp.float32
    out = pl.pallas_call(
        _kernel,
        out_shape=jax.ShapeDtypeStruct((D, S), bf),
        in_specs=[pl.BlockSpec(memory_space=pltpu.HBM)] * 6,
        out_specs=pl.BlockSpec(memory_space=pltpu.HBM),
        scratch_shapes=[
            pltpu.VMEM((D, S), bf),
            pltpu.VMEM((D, 3 * D), bf),
            pltpu.VMEM((D, D), bf),
            pltpu.VMEM((D, 1792), bf),
            pltpu.VMEM((D, DP), bf),
            pltpu.VMEM((D, F), bf),
            pltpu.VMEM((D, F), bf),
            pltpu.VMEM((D, F), bf),
            pltpu.VMEM((D, S), f32),
            pltpu.VMEM((S, D), bf),
            pltpu.VMEM((T, DP), f32),
            pltpu.VMEM((T + HALO, DP), f32),
            pltpu.VMEM((T + HALO, DP), f32),
            pltpu.VMEM((D, S), bf),
            pltpu.SemaphoreType.DMA((8,)),
        ],
        compiler_params=pltpu.CompilerParams(vmem_limit_bytes=100 * 1024 * 1024),
    )(x2, A_wqkv, A_wo, B_w_gate, B_w_up, B_w_down.T)
    return out.T.reshape(1, S, D)
```
